```python
import os as _os
_os.environ.setdefault("JAX_PLATFORMS", "cpu")
import jax
import jax.numpy as jnp

def _softmax(x, axis=-1):
    return jax.nn.softmax(x, axis=axis)
def _gelu(x):
    return jax.nn.gelu(x, approximate=True)
def _silu(x):
    return jax.nn.silu(x)
def _sigmoid(x):
    return jax.nn.sigmoid(x)
def _layernorm(x, axis=-1, eps=1e-5):
    m = jnp.mean(x, axis=axis, keepdims=True)
    v = jnp.var(x, axis=axis, keepdims=True)
    return (x - m) / jnp.sqrt(v + eps)
def _scatter_add(tgt, idx, src, axis=0):
    return tgt.at[idx].add(src)
def _segment_sum(src, seg, n):
    return jax.ops.segment_sum(src, seg, n)
class _Rng:
    def __init__(self, key):
        self._k = key
    def _next(self):
        self._k, sub = jax.random.split(self._k)
        return sub
    def normal(self, shape):
        return jax.random.normal(self._next(), shape, dtype=jnp.bfloat16)
    def randint(self, lo, hi, shape):
        return jax.random.randint(self._next(), shape, lo, hi, dtype=jnp.int32)
    def uniform(self, shape, lo=0.0, hi=1.0):
        return jax.random.uniform(self._next(), shape, jnp.bfloat16, lo, hi)
    def permutation(self, n):
        return jax.random.permutation(self._next(), n)


kernel_name = 'recurrent_scan__spectral_gfnet__swiglu_ffn__prompt'

def setup_inputs():
    _rng = _Rng(jax.random.key(int.from_bytes(__import__("os").urandom(4), "little")))
    _w = (lambda a: (lambda t: t.astype(jnp.bfloat16) if jnp.issubdtype(t.dtype, jnp.floating) else t)(jnp.asarray(a)))
    def _A_setup():
        B, S, D = 1, 2048, 640
        Df = D // 2 + 1
        return {
            "x": _w((lambda *s: _rng.normal(s) * 0.05)(B, S, D)),
            "w_r": _w((lambda *s: _rng.normal(s) * 0.05)(S, Df) * 0.02),
            "w_i": _w((lambda *s: _rng.normal(s) * 0.05)(S, Df) * 0.02),
        }
    _A_in = _A_setup()

    def _B_setup():
        B, S, D, F = 1, 2048, 640, 1536
        return {
            "x": _w((lambda *s: _rng.normal(s) * 0.05)(B, S, D)),
            "w_gate": _w((lambda *s: _rng.normal(s) * 0.05)(D, F)),
            "w_up": _w((lambda *s: _rng.normal(s) * 0.05)(D, F)),
            "w_down": _w((lambda *s: _rng.normal(s) * 0.05)(F, D)),
        }
    _B_in = _B_setup()

    return {
        "A_x": _A_in["x"],
        "A_w_r": _A_in["w_r"],
        "A_w_i": _A_in["w_i"],
        "B_x": _B_in["x"],
        "B_w_gate": _B_in["w_gate"],
        "B_w_up": _B_in["w_up"],
        "B_w_down": _B_in["w_down"],
    }

def reference(A_x, A_w_r, A_w_i, B_x, B_w_gate, B_w_up, B_w_down):
    def _A_ref(x, w_r, w_i):
        B, S, D = x.shape
        X = (lambda x, axes=(-2,-1): jnp.fft.rfft2(x.astype(jnp.float32), axes=axes))(x, axes=(-2, -1))
        W = w_r + 1j * w_i
        X = X * W
        y = (lambda x, s, axes=(-2,-1): jnp.fft.irfft2(x, s=s, axes=axes).astype(jnp.bfloat16))(X, (S, D), axes=(-2, -1))
        return y

    def _B_ref(x, w_gate, w_up, w_down):
        g = _silu(x @ w_gate)
        u = x @ w_up
        return (g * u) @ w_down

    x = A_x
    xn = _layernorm(x, axis=-1)
    s = _A_ref(xn, A_w_r, A_w_i)
    g = _silu(_B_ref(xn, B_w_gate, B_w_up, B_w_down))
    return x + s * g
```

```python
import functools
import math

import jax
import jax.numpy as jnp
import numpy as np
import jax.experimental.pallas as pl
import jax.experimental.pallas.tpu as pltpu

S, D, F = 2048, 640, 1536
DF = D // 2 + 1
R1, R2 = 32, 64
NT = 3
RB = 256
NB = S // RB
HB = 128
SB = 16
FC = 512
HC = 256
NC = F // FC
PLAN = ((0, 1, 2, 3, 4), (5, 6, 7), (8, 9, 10), (11, 12, 13, 14, 15))
assert sorted(sum(PLAN, ())) == list(range((NC - 1) * NB))
FINE = (True, True, True, False)
L0, LA, LB, LC, LD, LE = (2, 0, 0, 6), 5, 4, -2, 3, 1
DC = 4
SLOTS = 6


def _freq_columns():
    cols = -np.ones((NT, 128), np.int64)
    cols[0, :65] = 5 * np.arange(65)
    for t in (1, 2):
        cols[t] = np.concatenate([t + 5 * np.arange(64), 5 - t + 5 * np.arange(64)])
    return cols


def _constants():
    cols = _freq_columns()
    d2 = np.arange(128)[:, None]
    a0 = 2 * np.pi * d2 * cols[0, :65][None, :] / D
    m0 = np.concatenate([np.cos(a0), -np.sin(a0)[:, 1:64]], axis=1)
    wgt = np.where(np.arange(128) % 64 == 0, 1.0, 2.0)[None, :] / D
    dmat, nmat = [m0], [(m0 * wgt).T]
    for t in (1, 2):
        k = np.where(np.arange(128) < 64, cols[t], D - cols[t])
        a = 2 * np.pi * d2 * k[None, :] / D
        c, s = np.cos(a), np.sin(a)
        three = [c, s - c, -s - c]
        dmat += three
        nmat += [m.T * (2.0 / D) for m in three]
    dmat, nmat = 2.0 * np.stack(dmat), np.stack(nmat)
    n2 = np.arange(R2)[None, None, :]
    k = np.arange(R1)[:, None, None] + R1 * np.arange(R2)[None, :, None]
    a = 2 * np.pi * ((n2 * k) % S) / S
    c, s = np.cos(a), -np.sin(a)
    fmat = np.concatenate([np.concatenate([c, -s], axis=2), np.concatenate([s, c], axis=2)], axis=1)
    gmat = np.swapaxes(fmat, 1, 2) / S
    bf = jnp.bfloat16
    return dmat.astype(bf), nmat.astype(bf), fmat.astype(bf), gmat.astype(bf)


_DMAT, _NMAT, _FMAT, _GMAT = _constants()


def _twiddle(v, e, n, sign):
    re, im = v
    e %= n
    if sign < 0:
        e = (n - e) % n
    if e == 0:
        return re, im
    if 4 * e == n:
        return -im, re
    if 2 * e == n:
        return -re, -im
    if 4 * e == 3 * n:
        return im, -re
    c, s = math.cos(2 * math.pi * e / n), math.sin(2 * math.pi * e / n)
    if (8 * e) % n == 0:
        h = math.sqrt(0.5)
        q = (8 * e) // n
        if q == 1:
            return (re - im) * h, (re + im) * h
        if q == 3:
            return (re + im) * (-h), (re - im) * h
        if q == 5:
            return (im - re) * h, (re + im) * (-h)
        return (re + im) * h, (im - re) * h
    return re * c - im * s, re * s + im * c


def _fft(xs, sign):
    n = len(xs)
    if n == 1:
        return xs
    if n == 2:
        (ar, ai), (br, bi) = xs
        return [(ar + br, ai + bi), (ar - br, ai - bi)]
    ev = _fft(xs[0::2], sign)
    o1 = _fft(xs[1::4], sign)
    o3 = _fft(xs[3::4], sign)
    out = [None] * n
    q = n // 4
    for k in range(q):
        ar, ai = _twiddle(o1[k], k, n, sign)
        br, bi = _twiddle(o3[k], 3 * k, n, sign)
        sr, si, dr, di = ar + br, ai + bi, ar - br, ai - bi
        (er, ei), (fr, fi) = ev[k], ev[k + q]
        out[k] = (er + sr, ei + si)
        out[k + 2 * q] = (er - sr, ei - si)
        if sign < 0:
            out[k + q] = (fr + di, fi - dr)
            out[k + 3 * q] = (fr - di, fi + dr)
        else:
            out[k + q] = (fr - di, fi + dr)
            out[k + 3 * q] = (fr + di, fi - dr)
    return out


_C1, _C2 = math.cos(2 * math.pi / 5), math.cos(4 * math.pi / 5)
_S1, _S2 = math.sin(2 * math.pi / 5), math.sin(4 * math.pi / 5)


def _dot(a, b):
    return jnp.dot(a, b, preferred_element_type=jnp.float32)


def _silu_2x(h):
    return h + h * jnp.tanh(h)


def _radix5_even(z0, a, b):
    s = a + b
    m, n = z0 - 0.25 * s, (0.5 * (_C1 - _C2)) * (a - b)
    return z0 + s, m + n, m - n


def _spread(extras, lo=0, hi=8):
    return [(lo + (hi - lo) * n // len(extras), e) for n, e in enumerate(extras)]


def _interleave(main, extras, tick, clock, delay):
    res = []
    for n, step in enumerate(main):
        res.append(step())
        todo = [e for at, e in extras if at == n]
        for q, extra in enumerate(todo):
            if delay >= 0:
                tick(clock)
            elif n + delay >= 0:
                row = RB // 8 * q // len(todo) * 8
                tick(res[n + delay][row:row + 8, 0:128])
            extra()
            for _ in range(delay):
                clock = jnp.tanh(clock)


def _kernel(x_hbm, wr_hbm, wi_hbm, wg_hbm, wu_hbm, wd_hbm, dm_hbm, nm_hbm, fm_hbm, gm_hbm,
            o_hbm,
            x_v, xn_v, wr_v, wi_v, wp_v, wg_v, wu_v, wd_v, dm_v, nm_v, fm_v, gm_v, wt_v,
            buf_a, buf_b, tmp, acc, o_v, wsem, osem):
    f32, bf16, u32 = jnp.float32, jnp.bfloat16, jnp.uint32
    part = functools.partial

    def block(r):
        return pl.ds(pl.multiple_of(r * RB, RB), RB)

    def o_copy(r):
        return pltpu.make_async_copy(o_v.at[block(r)], o_hbm.at[block(r)], osem.at[r])

    def weight_pairs(c, lo, n):
        src, dst = pl.ds(c * FC + lo, n), pl.ds(lo, n)
        return [(wg_hbm.at[:, src], wg_v.at[c, :, dst]), (wu_hbm.at[:, src], wu_v.at[c, :, dst]),
                (wd_hbm.at[src, :], wd_v.at[c, dst, :])]

    def x_pair(lo, hi):
        return [(x_hbm.at[lo * RB:hi * RB], x_v.at[lo * RB:hi * RB])]

    half0, half1 = weight_pairs(0, 0, HC), weight_pairs(0, HC, HC)
    stages = [x_pair(0, 1) + half0[0:1], x_pair(1, 2) + half0[1:2], half0[2:3],
              half1[0:2] + [(dm_hbm, dm_v)], half1[2:3] + x_pair(2, 3), x_pair(3, NB), [],
              sum([weight_pairs(c, 0, FC) for c in range(1, NC)], [])
              + [(wr_hbm, wr_v), (wi_hbm, wi_v), (fm_hbm, fm_v), (gm_hbm, gm_v), (nm_hbm, nm_v)]]
    sems = iter(range(wsem.shape[0]))
    stages = [[pltpu.make_async_copy(a, b, wsem.at[next(sems)]) for a, b in st] for st in stages]
    rest = stages[-1]

    def ffn_unit(r, c, first_chunk, fine=False):
        rows, hs = block(r), {}

        def hidden(w_v, j, lo, hi):
            p = _dot(xn_v[rows, lo:hi], w_v[c, lo:hi, HC * j:HC * (j + 1)])
            key = (w_v is wu_v, j)
            hs[key] = hs[key] + p if lo else p
            if w_v is wu_v and hi == D:
                hs[j] = (_silu_2x(hs[False, j]) * hs[key]).astype(bf16)
            return p

        def down(j, lo, hi, k0, k1):
            p = _dot(hs[j][:, k0:k1], wd_v[c, HC * j + k0:HC * j + k1, lo:hi])
            hs[lo, hi] = hs[lo, hi] + p if k0 else p
            if k1 == HC:
                acc[rows, lo:hi] = hs[lo, hi] if first_chunk and j == 0 else acc[rows, lo:hi] + hs[lo, hi]
            return p

        kd, kh = (128, 128) if fine else (D, HC)
        order = ((0, 0, 256), (0, 256, D), (1, 0, 256), (1, 256, D))
        return ([part(hidden, w_v, j, k, k + kd) for j in range(FC // HC) for w_v in (wg_v, wu_v)
                 for k in range(0, D, kd)] + [part(down, *o, k, k + kh) for o in order for k in range(0, HC, kh)])

    def strip(r, q):
        return pl.ds(pl.multiple_of(r * RB + q * SB, SB), SB)

    def layernorm(r, q):
        xf = x_v[strip(r, q), :].astype(f32)
        xc = xf - jnp.mean(xf, axis=-1, keepdims=True)
        var = jnp.mean(xc * xc, axis=-1, keepdims=True)
        xn_v[strip(r, q), :] = (xc * (0.5 * jax.lax.rsqrt(var + 1e-5))).astype(bf16)

    def lane():
        return jax.lax.broadcasted_iota(jnp.int32, (1, 128), 1)

    def flip():
        return jnp.where(lane() < 64, 1.0, -1.0)

    def operands(*parts):
        return tuple(v.astype(bf16) for v in parts + ((parts[0] + parts[1],) if len(parts) == 2 else ()))

    def feature_dft(r):
        ys = [[], [], []]

        def butterfly(q):
            x0, x1, x2, x3, x4 = (xn_v[strip(r, q), 128 * t:128 * (t + 1)].astype(f32) for t in range(5))
            t1, t2, t3, t4 = x1 + x4, x2 + x3, x1 - x4, x2 - x3
            y0, y1, y2 = _radix5_even(x0, t1, t2)
            ys[0].append((y0,))
            ys[1].append((y1, -_S1 * t3 - _S2 * t4))
            ys[2].append((y2, _S1 * t4 - _S2 * t3))
            for y in ys:
                y[-1] = operands(*y[-1])

        def dft(t, h):
            y = [jnp.concatenate(v, axis=0) for v in zip(*ys[t][h * HB // SB:(h + 1) * HB // SB])]
            if t:
                both = _dot(y[2], dm_v[3 * t - 2])
                re, im = both + _dot(y[1], dm_v[3 * t - 1]), (both + _dot(y[0], dm_v[3 * t])) * flip()
            else:
                re = _dot(y[0], dm_v[0])
                im = jnp.where(lane() % 64 == 0, 0.0, pltpu.roll(re, 64, 1))
            for b in range(HB // R2):
                blk = r * (RB // R2) + h * (HB // R2) + b
                buf_a[blk, t, 0:R2, :] = re[R2 * b:R2 * (b + 1)]
                buf_a[blk, t, R2:, :] = im[R2 * b:R2 * (b + 1)]

        return [part(butterfly, q) for q in range(RB // SB)], [part(dft, t, h) for h in range(RB // HB) for t in range(NT)]

    def block_fft(j, t, m, sign):
        re_rows = pl.ds(pl.multiple_of(j * 8, 8), 8)
        im_rows = pl.ds(pl.multiple_of(j * 8 + R2, 8), 8)

        def eight(lo):
            ys = _fft([(buf_a[4 * a + lo, t, re_rows, :], buf_a[4 * a + lo, t, im_rows, :]) for a in range(8)], sign)
            for ka in range(8):
                tmp[m, ka, lo, 0], tmp[m, ka, lo, 1] = ys[ka]

        def four(ka):
            ys = _fft([_twiddle((tmp[m, ka, lo, 0], tmp[m, ka, lo, 1]), lo * ka, R1, sign) for lo in range(4)], sign)
            for kb in range(4):
                buf_b[ka + 8 * kb, t, re_rows, :], buf_b[ka + 8 * kb, t, im_rows, :] = ys[kb]

        return [part(eight, lo) for lo in range(4)], [part(four, ka) for ka in range(8)]

    def block_ffts(sign):
        units = [block_fft(j, t, (j * NT + t) % SLOTS, sign) for j in range(R2 // 8) for t in range(NT)]
        steps = list(units[0][0])
        for prev, cur in zip(units, units[1:]):
            for lo in range(4):
                steps += [cur[0][lo]] + prev[1][2 * lo:2 * lo + 2]
        return steps + units[-1][1]

    def filter_block(q, m):
        rows = pl.ds(pl.multiple_of(q * 128, 128), 128)
        re = pltpu.bitcast(wr_v[:, rows].astype(f32), u32)
        im = pltpu.bitcast(wi_v[:, rows].astype(f32), u32)
        wt_v[m, 0:DF, :] = re | (im >> 16)
        for t in range(NT):
            top = wt_v[m, pl.ds(t, 64, stride=5), :]
            bot = wt_v[m, pl.ds(5 - t, 64, stride=5), :] if t else wt_v[m, 320:384, :]
            wp_v[t, rows, :] = jnp.concatenate([top, bot], axis=0).T

    def spectral(k1, t):
        vals = []

        def forward():
            vals.append(_dot(fm_v[k1], buf_b[k1, t].astype(bf16)))
            w = wp_v[t, pl.ds(k1, R2, stride=R1), :]
            wr = pltpu.bitcast(w & jnp.uint32(0xFFFF0000), f32)
            wi = pltpu.bitcast(w << 16, f32)
            xr, xi = vals[0][0:R2], vals[0][R2:]
            vals.append(jnp.concatenate([xr * wr - xi * wi, xr * wi + xi * wr], axis=0).astype(bf16))

        def inverse():
            buf_a[k1, t] = _dot(gm_v[k1], vals[1])

        return forward, inverse

    def finish(r, h):
        nb, ns = HB // R2, HB // SB
        zs = {}

        def pack(t, b):
            re, im = buf_b[r * (RB // R2) + h * nb + b, t, 0:R2, :], buf_b[r * (RB // R2) + h * nb + b, t, R2:, :]
            zs[t, b] = operands(re, im * flip()) if t else operands(jnp.where(lane() <= 64, re, pltpu.roll(im, 64, 1)))

        def dft(t):
            y = [jnp.concatenate(v, axis=0) for v in zip(*[zs[t, b] for b in range(nb)])]
            if t:
                both = _dot(y[2], nm_v[3 * t - 2])
                zs[t] = (both + _dot(y[1], nm_v[3 * t]), both + _dot(y[0], nm_v[3 * t - 1]))
            else:
                zs[t] = (_dot(y[0], nm_v[0]),)

        def combine(q):
            z0, z1r, z1i, z2r, z2i = (z[SB * q:SB * (q + 1)] for t in range(NT) for z in zs[t])
            p0, p1, p2 = _radix5_even(z0, z1r, z2r)
            q1 = _S1 * z1i + _S2 * z2i
            q2 = _S2 * z1i - _S1 * z2i
            zs["s", q] = (p0, p1 - q1, p2 - q2, p2 + q2, p1 + q1)

        def emit(q, t):
            rows, cols = strip(r, h * ns + q), slice(128 * t, 128 * (t + 1))
            o_v[rows, cols] = (x_v[rows, cols].astype(f32) + zs["s", q][t] * _silu_2x(acc[rows, cols])).astype(bf16)

        strips = range(ns)
        return ([part(pack, t, b) for t in range(NT) for b in range(nb)], [part(dft, t) for t in range(NT)],
                [part(combine, q) for q in strips], [[part(emit, q, t) for q in strips] for t in range(D // 128)])

    def clock0():
        return xn_v[0:16, 0:128].astype(f32)[0:8]

    def start(cps):
        for cp in cps:
            cp.start()

    def wait(cps):
        for cp in cps:
            cp.wait()

    def tick_a(slot, v):
        spare = pl.ds(pl.multiple_of(S + 16 * slot, 16), 16)
        x_v[spare, 0:128] = jnp.concatenate([v, v], axis=0).astype(bf16)

    def norms(r):
        return [part(layernorm, r, q) for q in range(RB // SB)]

    def phase_a(r, carry):
        bfly, dfts = feature_dft(r)
        extras = _spread(bfly, 0, 3) + _spread(dfts, 4, 7) + _spread(norms(jnp.minimum(r + 1, NB - 1)), 3, 8)
        _interleave(ffn_unit(r, 0, True), extras, part(tick_a, zero), clock0(), LA)
        return carry

    def stage(n):
        wait(stages[n])
        start(stages[n + 2])

    start(stages[0] + stages[1])

    def clear(m, carry):
        wt_v[m, 320:384, :] = jnp.zeros((64, 128), u32)
        return wt_v.shape[0] - 1 - m

    zero = jax.lax.fori_loop(0, wt_v.shape[0], clear, 0)
    stage(0)
    f0, f1 = ffn_unit(0, 0, True), ffn_unit(1, 0, True)
    (bfly0, dft0), (bfly1, dft1) = feature_dft(0), feature_dft(1)
    for q in range(RB // SB):
        layernorm(0, q)
    f0[0]()
    for n, (main, extras) in enumerate((
            (f0[1:2] + f1[0:2], _spread(norms(1), 0, 1)),
            (f0[4:6] + f1[4:6], _spread(bfly0, 0, 4)),
            (f0[2:4] + f1[2:4], _spread(bfly1, 0, 4) + _spread(dft0, 1, 4)),
            (f0[6:8] + f1[6:8], _spread(norms(2), 0, 4) + _spread(dft1, 0, 3)))):
        stage(n + 1)
        _interleave(main, extras, part(tick_a, zero), clock0(), L0[n])
    stage(5)

    def ffn_steps(phase):
        return sum([ffn_unit(u % NB, 1 + u // NB, False, FINE[phase]) for u in PLAN[phase]], [])

    def tick(pace, v):
        pace[R1 + zero, 0, 0:8, :] = v
        if pace is buf_a:
            tmp[SLOTS + zero, 0, 0, 0] = v

    def phase_b():
        main = ffn_steps(0)
        filt = [part(filter_block, q, q % wt_v.shape[0]) for q in range(S // 128)]
        extras = _spread(block_ffts(-1), 0, len(main)) + _spread(filt, 0, len(main) * 7 // 8)
        _interleave(main, extras, part(tick, buf_a), clock0(), LB)

    def phase_c():
        main = ffn_steps(1)
        units = [spectral(k1, t) for k1 in range(R1) for t in range(NT)]
        order = [units[n - d][p] for n in range(len(units) + DC) for p, d in enumerate((0, DC))
                 if 0 <= n - d < len(units)]
        _interleave(main, _spread(order, 0, len(main)), part(tick, buf_b), clock0(), LC)

    def phase_d():
        main = ffn_steps(2)
        _interleave(main, _spread(block_ffts(1), 0, len(main)), part(tick, buf_a), clock0(), LD)

    def phase_e():
        main = ffn_steps(3)
        extras, late, nh = [], [], RB // HB
        for n in range(NB * nh):
            pack, dft, mix, emit = finish(n // nh, n % nh)
            at = n * (len(main) - 4) // (NB * nh)
            last = (NC - 2) * NB + n // nh
            ready = 8 * PLAN[3].index(last) + 7 if last in PLAN[3] else 0
            extras += _spread(pack, at, at + 1)
            late += _spread(dft, at, at + 1)
            if ready > at + 1:
                extras += (_spread(mix, at + 1, at + 2) + _spread(emit[0] + emit[1], ready - 1, ready)
                           + _spread(emit[2] + emit[3] + emit[4], ready, ready + 1))
            else:
                extras += _spread(sum([[m] + list(e) for m, e in zip(mix, zip(*emit))], []), at + 1, at + 2)
            if n % nh == nh - 1:
                late += [(min(max(at + 3, ready), len(main) - 1), o_copy(n // nh).start)]
        _interleave(main, extras + late, part(tick, buf_b), clock0(), LE)

    jax.lax.fori_loop(2, NB, phase_a, 0)
    for cp in rest:
        cp.wait()
    for n, body in enumerate((phase_b, phase_c, phase_d, phase_e)):
        pl.when(zero <= n)(body)
    for r in range(NB):
        o_copy(r).wait()


@jax.jit
def pallas_recurrent_scan__spectral_gfnet__swiglu_ffn__prompt_kernel(
    A_x: jax.Array,
    A_w_r: jax.Array,
    A_w_i: jax.Array,
    B_x: jax.Array,
    B_w_gate: jax.Array,
    B_w_up: jax.Array,
    B_w_down: jax.Array,
):
    del B_x
    bf16, f32 = jnp.bfloat16, jnp.float32
    hbm = pl.BlockSpec(memory_space=pltpu.HBM)
    out = pl.pallas_call(
        _kernel,
        out_shape=jax.ShapeDtypeStruct((S, D), bf16),
        in_specs=[hbm] * 10,
        out_specs=hbm,
        scratch_shapes=[
            pltpu.VMEM((S + 16, D), bf16), pltpu.VMEM((S, D), bf16),
            pltpu.VMEM((DF, S), bf16), pltpu.VMEM((DF, S), bf16), pltpu.VMEM((NT, S + R1, 128), jnp.uint32),
            pltpu.VMEM((NC, D, FC), bf16), pltpu.VMEM((NC, D, FC), bf16), pltpu.VMEM((NC, FC, D), bf16),
            pltpu.VMEM(_DMAT.shape, bf16), pltpu.VMEM(_NMAT.shape, bf16),
            pltpu.VMEM(_FMAT.shape, bf16), pltpu.VMEM(_GMAT.shape, bf16), pltpu.VMEM((4, NT * 128, 128), jnp.uint32),
            pltpu.VMEM((R1 + 1, NT, 2 * R2, 128), f32), pltpu.VMEM((R1 + 1, NT, 2 * R2, 128), f32),
            pltpu.VMEM((SLOTS + 1, 8, 4, 2, 8, 128), f32), pltpu.VMEM((S, D), f32), pltpu.VMEM((S, D), bf16),
            pltpu.SemaphoreType.DMA((3 * NC + 13,)),
            pltpu.SemaphoreType.DMA((NB,)),
        ],
        compiler_params=pltpu.CompilerParams(vmem_limit_bytes=124 * 1024 * 1024),
    )(A_x.reshape(S, D), A_w_r.T, A_w_i.T, B_w_gate, B_w_up, B_w_down, _DMAT, _NMAT, _FMAT, _GMAT)
    return out.reshape(A_x.shape)
```
